```python
import os as _os
_os.environ.setdefault("JAX_PLATFORMS", "cpu")
import jax
import jax.numpy as jnp

def _softmax(x, axis=-1):
    return jax.nn.softmax(x, axis=axis)
def _gelu(x):
    return jax.nn.gelu(x, approximate=True)
def _silu(x):
    return jax.nn.silu(x)
def _sigmoid(x):
    return jax.nn.sigmoid(x)
def _layernorm(x, axis=-1, eps=1e-5):
    m = jnp.mean(x, axis=axis, keepdims=True)
    v = jnp.var(x, axis=axis, keepdims=True)
    return (x - m) / jnp.sqrt(v + eps)
def _scatter_add(tgt, idx, src, axis=0):
    return tgt.at[idx].add(src)
def _segment_sum(src, seg, n):
    return jax.ops.segment_sum(src, seg, n)
class _Rng:
    def __init__(self, key):
        self._k = key
    def _next(self):
        self._k, sub = jax.random.split(self._k)
        return sub
    def normal(self, shape):
        return jax.random.normal(self._next(), shape, dtype=jnp.bfloat16)
    def randint(self, lo, hi, shape):
        return jax.random.randint(self._next(), shape, lo, hi, dtype=jnp.int32)
    def uniform(self, shape, lo=0.0, hi=1.0):
        return jax.random.uniform(self._next(), shape, jnp.bfloat16, lo, hi)
    def permutation(self, n):
        return jax.random.permutation(self._next(), n)


kernel_name = 'gated_mix__gqa_block_cached__dense_activation_squared_relu__decode'

def setup_inputs():
    _rng = _Rng(jax.random.key(int.from_bytes(__import__("os").urandom(4), "little")))
    _w = (lambda a: (lambda t: t.astype(jnp.bfloat16) if jnp.issubdtype(t.dtype, jnp.floating) else t)(jnp.asarray(a)))
    def _A_setup():
        B, Sq, D = 4, 1, 512
        Hq, Hkv, Sk, Dh = 32, 8, 4096, 128
        assert Hq % Hkv == 0, (Hq, Hkv)
        return {
            "x": _w((lambda *s: _rng.normal(s) * 0.05)(B, Sq, D)),
            "k_cache": _w((lambda *s: _rng.normal(s) * 3.2)(B, Hkv, Sk, Dh)),
            "v_cache": _w((lambda *s: _rng.normal(s) * 1.6)(B, Hkv, Sk, Dh)),
            "wq": _w((lambda *s: _rng.normal(s) * 3.2)(D, Hq * Dh) * (D ** -0.5)),
            "wo": _w((lambda *s: _rng.normal(s) * 1.6)(Hq * Dh, D) * ((Hq * Dh) ** -0.5)),
        }
    _A_in = _A_setup()

    def _B_setup():
        B, S, D, F = 4, 1, 512, 1792
        return {
            "x": _w((lambda *s: _rng.normal(s) * 0.05)(B, S, D)),
            "w1": _w((lambda *s: _rng.normal(s) * 0.1)(D, F)),
            "b1": _w((lambda *s: _rng.normal(s) * 0.05)(F)),
            "w2": _w((lambda *s: _rng.normal(s) * 0.05)(F, D)),
            "b2": _w((lambda *s: _rng.normal(s) * 0.05)(D)),
        }
    _B_in = _B_setup()

    return {
        "A_x": _A_in["x"],
        "A_k_cache": _A_in["k_cache"],
        "A_v_cache": _A_in["v_cache"],
        "A_wq": _A_in["wq"],
        "A_wo": _A_in["wo"],
        "B_x": _B_in["x"],
        "B_w1": _B_in["w1"],
        "B_b1": _B_in["b1"],
        "B_w2": _B_in["w2"],
        "B_b2": _B_in["b2"],
        "gate_w": _w((lambda *s: _rng.normal(s) * 0.05)(512) * 16.0),
    }

def reference(A_x, A_k_cache, A_v_cache, A_wq, A_wo, B_x, B_w1, B_b1, B_w2, B_b2, gate_w):
    def _A_ref(x, k_cache, v_cache, wq, wo):
        B, Sq, D = x.shape
        Hq, Dh = 32, 128
        Hkv = k_cache.shape[1]
        rep = Hq // Hkv
        q = (lambda x, *d: x.transpose(*d))((x @ wq).reshape(B, Sq, Hq, Dh), 0, 2, 1, 3)
        k = jnp.repeat(k_cache, rep, axis=1)
        v = jnp.repeat(v_cache, rep, axis=1)
        scores = jnp.einsum("bhqd,bhkd->bhqk", q, k) * (Dh ** -0.5)
        p = _softmax(scores, axis=-1)
        o = jnp.einsum("bhqk,bhkd->bhqd", p, v)
        return (lambda x, *d: x.transpose(*d))(o, 0, 2, 1, 3).reshape(B, Sq, Hq * Dh) @ wo

    def _B_ref(x, w1, b1, w2, b2):
        h = jnp.einsum("bsd,df->bsf", x, w1) + b1
        zero = jnp.zeros_like(h)
        r = jnp.where(h > zero, h, zero)
        h = r * r
        out = jnp.einsum("bsf,fd->bsd", h, w2) + b2
        return out

    x = A_x
    g = _sigmoid((x * gate_w).sum(-1, keepdims=True))
    a = _A_ref(x, A_k_cache, A_v_cache, A_wq, A_wo)
    b = _B_ref(x, B_w1, B_b1, B_w2, B_b2)
    return g * a + (1 - g) * b
```

```python
import functools

import jax
import jax.numpy as jnp
from jax import lax
import jax.experimental.pallas as pl
import jax.experimental.pallas.tpu as pltpu


def _kernel(x_ref, gw_ref, wq_ref, k_ref, v_ref, wo_ref, w1_ref, b1_ref, w2_ref,
            b2_ref, out_ref, q_scr, o_scr, acc_scr, ffn_scr, *, rep, dh, scale):
    h = pl.program_id(0)
    b = pl.program_id(1)
    nh = pl.num_programs(0)
    nb = pl.num_programs(1)
    B = x_ref.shape[0]
    f32 = jnp.float32
    bf16 = jnp.bfloat16

    @pl.when(b == 0)
    def _():
        x = x_ref[...]
        for r in range(rep):
            qr = jnp.dot(x, wq_ref[:, r * dh:(r + 1) * dh],
                         preferred_element_type=f32)
            for bb in range(B):
                q_scr[bb, r:r + 1, :] = qr[bb:bb + 1, :]

    @pl.when(jnp.logical_and(h == 0, b == 1))
    def _():
        x = x_ref[...]
        hh = jnp.dot(x, w1_ref[...], preferred_element_type=f32)
        hh = hh + b1_ref[...].astype(f32)
        rr = jnp.maximum(hh, 0.0)
        hh = rr * rr
        y = jnp.dot(hh.astype(bf16), w2_ref[...], preferred_element_type=f32)
        ffn_scr[...] = y + b2_ref[...].astype(f32)

    q = q_scr[b].astype(bf16)
    k = k_ref[...]
    s = lax.dot_general(q, k, (((1,), (1,)), ((), ())),
                        preferred_element_type=f32) * scale
    m = jnp.max(s, axis=-1, keepdims=True)
    p = jnp.exp(s - m)
    l = jnp.sum(p, axis=-1, keepdims=True)
    o = jnp.dot(p.astype(bf16), v_ref[...], preferred_element_type=f32)
    o_scr[b] = o / l

    @pl.when(b == nb - 1)
    def _():
        part = None
        for r in range(rep):
            rows = [o_scr[bb, r:r + 1, :] for bb in range(B)]
            o_r = jnp.concatenate(rows, axis=0).astype(bf16)
            t = jnp.dot(o_r, wo_ref[r * dh:(r + 1) * dh, :],
                        preferred_element_type=f32)
            part = t if part is None else part + t

        @pl.when(h == 0)
        def _():
            acc_scr[...] = part

        @pl.when(h > 0)
        def _():
            acc_scr[...] = acc_scr[...] + part

    @pl.when(jnp.logical_and(h == nh - 1, b == nb - 1))
    def _():
        x = x_ref[...].astype(f32)
        gl = jnp.sum(x * gw_ref[...].astype(f32), axis=-1, keepdims=True)
        g = jax.nn.sigmoid(gl)
        out_ref[...] = (g * acc_scr[...] + (1.0 - g) * ffn_scr[...]).astype(out_ref.dtype)


@jax.jit
def pallas_gated_mix__gqa_block_cached__dense_activation_squared_relu__decode_kernel(
    A_x: jax.Array,
    A_k_cache: jax.Array,
    A_v_cache: jax.Array,
    A_wq: jax.Array,
    A_wo: jax.Array,
    B_x: jax.Array,
    B_w1: jax.Array,
    B_b1: jax.Array,
    B_w2: jax.Array,
    B_b2: jax.Array,
    gate_w: jax.Array,
):
    del B_x
    B, Sq, D = A_x.shape
    _, Hkv, Sk, Dh = A_k_cache.shape
    Hq = A_wq.shape[1] // Dh
    rep = Hq // Hkv
    F = B_w1.shape[1]
    assert Sq == 1

    x2 = A_x.reshape(B * Sq, D)
    gw2 = gate_w.reshape(1, D)
    b12 = B_b1.reshape(1, F)
    b22 = B_b2.reshape(1, D)

    hw = rep * Dh

    kernel = functools.partial(_kernel, rep=rep, dh=Dh, scale=float(Dh) ** -0.5)

    out = pl.pallas_call(
        kernel,
        out_shape=jax.ShapeDtypeStruct((B, D), A_x.dtype),
        grid=(Hkv, B),
        in_specs=[
            pl.BlockSpec((B, D), lambda h, b: (0, 0)),
            pl.BlockSpec((1, D), lambda h, b: (0, 0)),
            pl.BlockSpec((D, hw), lambda h, b: (0, h)),
            pl.BlockSpec((None, None, Sk, Dh), lambda h, b: (b, h, 0, 0)),
            pl.BlockSpec((None, None, Sk, Dh), lambda h, b: (b, h, 0, 0)),
            pl.BlockSpec((hw, D), lambda h, b: (h, 0)),
            pl.BlockSpec((D, F), lambda h, b: (0, 0)),
            pl.BlockSpec((1, F), lambda h, b: (0, 0)),
            pl.BlockSpec((F, D), lambda h, b: (0, 0)),
            pl.BlockSpec((1, D), lambda h, b: (0, 0)),
        ],
        out_specs=pl.BlockSpec((B, D), lambda h, b: (0, 0)),
        scratch_shapes=[
            pltpu.VMEM((B, rep, Dh), jnp.float32),
            pltpu.VMEM((B, rep, Dh), jnp.float32),
            pltpu.VMEM((B, D), jnp.float32),
            pltpu.VMEM((B, D), jnp.float32),
        ],
        compiler_params=pltpu.CompilerParams(
            dimension_semantics=("arbitrary", "arbitrary"),
            vmem_limit_bytes=64 * 1024 * 1024,
        ),
    )(x2, gw2, A_wq, A_k_cache, A_v_cache, A_wo, B_w1, b12, B_w2, b22)
    return out.reshape(B, Sq, D)
```

```python
import functools

import jax
import jax.numpy as jnp
from jax import lax
import jax.experimental.pallas as pl
import jax.experimental.pallas.tpu as pltpu


def _kernel(k_ref, v_ref, wq_ref, wo_ref, w1_ref, w2_ref, x_ref, gw_ref, b1_ref,
            b2_ref, out_ref, q_scr, o_scr, acc_scr, ffn_scr, g_scr,
            *, rep, dh, scale):
    h = pl.program_id(0)
    b = pl.program_id(1)
    nh = pl.num_programs(0)
    nb = pl.num_programs(1)
    B = x_ref.shape[0]
    f32 = jnp.float32
    bf16 = jnp.bfloat16

    @pl.when(b == 0)
    def _():
        x = x_ref[...]
        for r in range(rep):
            qr = jnp.dot(x, wq_ref[:, r * dh:(r + 1) * dh],
                         preferred_element_type=f32)
            for bb in range(B):
                q_scr[bb, r:r + 1, :] = qr[bb:bb + 1, :]

    @pl.when(jnp.logical_and(h == 0, b == 1))
    def _():
        x = x_ref[...]
        hh = jnp.dot(x, w1_ref[...], preferred_element_type=f32)
        hh = hh + b1_ref[...].astype(f32).reshape(1, -1)
        rr = jnp.maximum(hh, 0.0)
        hh = rr * rr
        y = jnp.dot(hh.astype(bf16), w2_ref[...], preferred_element_type=f32)
        y = y + b2_ref[...].astype(f32).reshape(1, -1)
        gl = jnp.sum(x.astype(f32) * gw_ref[...].astype(f32).reshape(1, -1),
                     axis=-1, keepdims=True)
        g = jax.nn.sigmoid(gl)
        g_scr[...] = jnp.broadcast_to(g, g_scr.shape)
        ffn_scr[...] = (1.0 - g) * y

    q = q_scr[b].astype(bf16)
    s = lax.dot_general(q, k_ref[...], (((1,), (1,)), ((), ())),
                        preferred_element_type=f32) * scale
    m = jnp.max(s, axis=-1, keepdims=True)
    p = jnp.exp(s - m)
    l = jnp.sum(p, axis=-1, keepdims=True)
    o = jnp.dot(p.astype(bf16), v_ref[...], preferred_element_type=f32)
    o_scr[b] = o / l

    @pl.when(b == nb - 1)
    def _():
        part = None
        for r in range(rep):
            rows = [o_scr[bb, r:r + 1, :] for bb in range(B)]
            o_r = jnp.concatenate(rows, axis=0).astype(bf16)
            t = jnp.dot(o_r, wo_ref[r * dh:(r + 1) * dh, :],
                        preferred_element_type=f32)
            part = t if part is None else part + t

        @pl.when(h == 0)
        def _():
            acc_scr[...] = part

        @pl.when(jnp.logical_and(h > 0, h < nh - 1))
        def _():
            acc_scr[...] = acc_scr[...] + part

        @pl.when(h == nh - 1)
        def _():
            a = acc_scr[...] + part
            out_ref[...] = (g_scr[...] * a + ffn_scr[...]).astype(out_ref.dtype)


@jax.jit
def pallas_gated_mix__gqa_block_cached__dense_activation_squared_relu__decode_kernel(
    A_x: jax.Array,
    A_k_cache: jax.Array,
    A_v_cache: jax.Array,
    A_wq: jax.Array,
    A_wo: jax.Array,
    B_x: jax.Array,
    B_w1: jax.Array,
    B_b1: jax.Array,
    B_w2: jax.Array,
    B_b2: jax.Array,
    gate_w: jax.Array,
):
    del B_x
    B, Sq, D = A_x.shape
    _, Hkv, Sk, Dh = A_k_cache.shape
    Hq = A_wq.shape[1] // Dh
    rep = Hq // Hkv
    F = B_w1.shape[1]
    assert Sq == 1 and Hkv > 1 and B > 1

    x2 = A_x.reshape(B * Sq, D)
    hw = rep * Dh

    kernel = functools.partial(_kernel, rep=rep, dh=Dh, scale=float(Dh) ** -0.5)

    out = pl.pallas_call(
        kernel,
        out_shape=jax.ShapeDtypeStruct((B, D), A_x.dtype),
        grid=(Hkv, B),
        in_specs=[
            pl.BlockSpec((None, None, Sk, Dh), lambda h, b: (b, h, 0, 0)),
            pl.BlockSpec((None, None, Sk, Dh), lambda h, b: (b, h, 0, 0)),
            pl.BlockSpec((D, hw), lambda h, b: (0, h)),
            pl.BlockSpec((hw, D), lambda h, b: (h, 0)),
            pl.BlockSpec((D, F), lambda h, b: (0, 0)),
            pl.BlockSpec((F, D), lambda h, b: (0, 0)),
            pl.BlockSpec((B, D), lambda h, b: (0, 0)),
            pl.BlockSpec((D,), lambda h, b: (0,)),
            pl.BlockSpec((F,), lambda h, b: (0,)),
            pl.BlockSpec((D,), lambda h, b: (0,)),
        ],
        out_specs=pl.BlockSpec((B, D), lambda h, b: (0, 0)),
        scratch_shapes=[
            pltpu.VMEM((B, rep, Dh), jnp.float32),
            pltpu.VMEM((B, rep, Dh), jnp.float32),
            pltpu.VMEM((B, D), jnp.float32),
            pltpu.VMEM((B, D), jnp.float32),
            pltpu.VMEM((B, D), jnp.float32),
        ],
        compiler_params=pltpu.CompilerParams(
            dimension_semantics=("arbitrary", "arbitrary"),
            vmem_limit_bytes=64 * 1024 * 1024,
        ),
    )(A_k_cache, A_v_cache, A_wq, A_wo, B_w1, B_w2, x2, gate_w, B_b1, B_b2)
    return out.reshape(B, Sq, D)
```
